```python
import os as _os
_os.environ.setdefault("JAX_PLATFORMS", "cpu")
import jax
import jax.numpy as jnp

def _softmax(x, axis=-1):
    return jax.nn.softmax(x, axis=axis)
def _gelu(x):
    return jax.nn.gelu(x, approximate=True)
def _silu(x):
    return jax.nn.silu(x)
def _sigmoid(x):
    return jax.nn.sigmoid(x)
def _layernorm(x, axis=-1, eps=1e-5):
    m = jnp.mean(x, axis=axis, keepdims=True)
    v = jnp.var(x, axis=axis, keepdims=True)
    return (x - m) / jnp.sqrt(v + eps)
def _scatter_add(tgt, idx, src, axis=0):
    return tgt.at[idx].add(src)
def _segment_sum(src, seg, n):
    return jax.ops.segment_sum(src, seg, n)
class _Rng:
    def __init__(self, key):
        self._k = key
    def _next(self):
        self._k, sub = jax.random.split(self._k)
        return sub
    def normal(self, shape):
        return jax.random.normal(self._next(), shape, dtype=jnp.bfloat16)
    def randint(self, lo, hi, shape):
        return jax.random.randint(self._next(), shape, lo, hi, dtype=jnp.int32)
    def uniform(self, shape, lo=0.0, hi=1.0):
        return jax.random.uniform(self._next(), shape, jnp.bfloat16, lo, hi)
    def permutation(self, n):
        return jax.random.permutation(self._next(), n)


kernel_name = 'standalone__channel_attn_cbam__vision'

def setup_inputs():
    _rng = _Rng(jax.random.key(int.from_bytes(__import__("os").urandom(4), "little")))
    _w = (lambda a: (lambda t: t.astype(jnp.bfloat16) if jnp.issubdtype(t.dtype, jnp.floating) else t)(jnp.asarray(a)))
    H = W = 384
    C = 192
    r = max(C // 4, 1)
    return {
        "x": _w((lambda *s: _rng.normal(s) * 0.2)(1, H, W, C) + (lambda *s: _rng.normal(s) * 0.2)(1, 1, 1, C) * 2.0),
        "w1": _w((lambda *s: _rng.normal(s) * 0.2)(C, r)),
        "w2": _w((lambda *s: _rng.normal(s) * 0.2)(r, C)),
    }

def reference(x, w1, w2):
    B, H, W, C = x.shape
    xf = x.reshape(B, H * W, C)
    gap = jnp.mean(xf, 1)
    gmp = jnp.amax(xf, 1)
    h_a = gap @ w1
    h_a = h_a * (lambda x, dt: x.astype(dt))(h_a > 0, h_a.dtype)
    h_m = gmp @ w1
    h_m = h_m * (lambda x, dt: x.astype(dt))(h_m > 0, h_m.dtype)
    scale = _sigmoid(h_a @ w2 + h_m @ w2)
    return x * scale[:, None, None, :]
```

```python
import functools

import jax
import jax.numpy as jnp
from jax import lax
import jax.experimental.pallas as pl
import jax.experimental.pallas.tpu as pltpu

LANES = 128
TILE = 8
RUN = 64
RD_STREAMS = 12
RD_PER_DMA = 2
RD_WINDOW = 12
WR_STREAMS = 6
WR_DIST = 64


def _kernel(x_hbm, w1t_hbm, w2_hbm, o_hbm, buf, wbuf, wt, acc_s, acc_m, tab, rsem, wsem, osem,
            *, hw, w_tiles):
    n_rounds = x_hbm.shape[1]
    hidden, C = w2_hbm.shape
    nq = C * w_tiles // RUN
    n_dma = RD_STREAMS // RD_PER_DMA
    f32 = jnp.float32

    def rd_start(r, slot, p):
        idx = (pl.ds(p * RD_PER_DMA, RD_PER_DMA), r)
        pltpu.make_async_copy(x_hbm.at[idx], buf.at[idx], rsem.at[slot]).start(priority=p % 2)

    def rd_wait(r, slot):
        pltpu.make_async_copy(x_hbm.at[:, r], buf.at[:, r], rsem.at[slot]).wait()

    def prologue(r, _):
        for p in range(n_dma):
            rd_start(r, r, p)

    lax.fori_loop(0, 2, prologue, None)
    w_copies = [pltpu.make_async_copy(w, wbuf.at[i], wsem) for i, w in enumerate((w1t_hbm, w2_hbm))]
    for c in w_copies:
        c.start()
    lax.fori_loop(2, RD_WINDOW, prologue, None)

    acc_s[...] = jnp.zeros(acc_s.shape, f32)
    acc_m[...] = jnp.full(acc_m.shape, -jnp.inf, f32)
    for c in w_copies:
        c.wait()
    for i in range(2):
        w = wbuf[i].astype(f32)
        w = jnp.concatenate([w, jnp.zeros((hidden, 2 * LANES - C), f32)], axis=1)
        w = jnp.concatenate([w, jnp.zeros((LANES - hidden, 2 * LANES), f32)], axis=0)
        wt[i] = w.T[:C]

    def reduce_round(r, q, slot, refill):
        rd_wait(r, slot)
        s, m = acc_s[q], acc_m[q]
        for p in range(n_dma):
            if refill:
                rd_start(r + RD_WINDOW, slot, p)
            for st in range(p * RD_PER_DMA, (p + 1) * RD_PER_DMA):
                v = buf[st, r].astype(f32)
                s, m = s + v, jnp.maximum(m, v)
        return s, m

    def loop(refill):
        def body(r, carry):
            q, slot = carry
            acc_s[q], acc_m[q] = reduce_round(r, q, slot, refill)
            q = jnp.where(q == nq - 1, 0, q + 1)
            slot = jnp.where(slot == RD_WINDOW - 1, 0, slot + 1)
            return q, slot
        return body

    carry = (jnp.int32(0), jnp.int32(0))
    carry = lax.fori_loop(0, n_rounds - RD_WINDOW, loop(True), carry)
    lax.fori_loop(n_rounds - RD_WINDOW, n_rounds - nq, loop(False), carry)

    def rnd(v):
        return v.astype(jnp.bfloat16).astype(f32)

    ha = jnp.zeros((TILE, LANES), f32)
    hm = jnp.zeros((TILE, LANES), f32)
    ts, tm = [], []
    for q in range(nq):
        r = n_rounds - nq + q
        s, m = reduce_round(r, q, r % RD_WINDOW, False)
        for i in range(RUN // TILE):
            ts.append(s[i * TILE:(i + 1) * TILE])
            tm.append(m[i * TILE:(i + 1) * TILE])
            if len(ts) % w_tiles == 0:
                g = len(ts) // w_tiles - 1
                gs = functools.reduce(jnp.add, ts[-w_tiles:])
                gm = functools.reduce(jnp.maximum, tm[-w_tiles:])
                gap = rnd(jnp.sum(gs, axis=1, keepdims=True) * (1.0 / hw))
                gmp = jnp.max(gm, axis=1, keepdims=True)
                w = wt[0, g * TILE:(g + 1) * TILE]
                ha, hm = ha + gap * w, hm + gmp * w

    def act(h):
        h = rnd(jnp.sum(h, axis=0, keepdims=True))
        return h * (h > 0).astype(f32)

    lane = lax.broadcasted_iota(jnp.int32, (1, LANES), 1)
    h = jnp.where(lane < hidden, act(ha) + act(hm), 0.0)
    z = jnp.sum(wt[1] * h, axis=1, keepdims=True)
    scale = jnp.broadcast_to(rnd(jax.nn.sigmoid(z)), (C, LANES))
    for t in range(C * w_tiles // TILE):
        g = t // w_tiles
        tab[t * TILE // RUN, pl.ds(t * TILE % RUN, TILE)] = scale[g * TILE:(g + 1) * TILE]

    obuf = buf.reshape(*o_hbm.shape)
    n_blocks = o_hbm.shape[0] // WR_STREAMS

    def write_step(i, _):
        b, g = i // WR_DIST, i % WR_DIST
        q = (b * WR_STREAMS * WR_DIST + g) % nq
        for st in range(WR_STREAMS):
            u = b * WR_STREAMS + st
            obuf[u, g] = (obuf[u, g].astype(f32) * tab[q]).astype(obuf.dtype)
            q = q + WR_DIST % nq
            q = jnp.where(q >= nq, q - nq, q)
        idx = (pl.ds(b * WR_STREAMS, WR_STREAMS), g)
        pltpu.make_async_copy(obuf.at[idx], o_hbm.at[idx], osem).start()

    lax.fori_loop(0, n_blocks * WR_DIST, write_step, None)
    pltpu.make_async_copy(obuf, o_hbm, osem).wait()


@jax.jit
def pallas_standalone__channel_attn_cbam__vision_kernel(
    x: jax.Array,
    w1: jax.Array,
    w2: jax.Array,
):
    B, H, W, C = x.shape
    hidden = w1.shape[1]
    assert B == 1
    w_tiles = W // LANES
    n_runs = H * C * w_tiles // RUN
    nq = C * w_tiles // RUN
    rd_shape = (RD_STREAMS, n_runs // RD_STREAMS, RUN, LANES)
    wr_shape = (n_runs // WR_DIST, WR_DIST, RUN, LANES)

    xl = x.reshape(H, w_tiles, LANES, C // TILE, TILE).transpose(0, 3, 1, 4, 2).reshape(rd_shape)
    hbm = pl.BlockSpec(memory_space=pltpu.HBM)
    out = pl.pallas_call(
        functools.partial(_kernel, hw=H * W, w_tiles=w_tiles),
        out_shape=jax.ShapeDtypeStruct(wr_shape, x.dtype),
        in_specs=[hbm, hbm, hbm],
        out_specs=hbm,
        scratch_shapes=[
            pltpu.VMEM(rd_shape, x.dtype),
            pltpu.VMEM((2, hidden, C), w1.dtype),
            pltpu.VMEM((2, C, LANES), jnp.float32),
            pltpu.VMEM((nq, RUN, LANES), jnp.float32),
            pltpu.VMEM((nq, RUN, LANES), jnp.float32),
            pltpu.VMEM((nq, RUN, LANES), jnp.float32),
            pltpu.SemaphoreType.DMA((RD_WINDOW,)),
            pltpu.SemaphoreType.DMA(()),
            pltpu.SemaphoreType.DMA(()),
        ],
        compiler_params=pltpu.CompilerParams(vmem_limit_bytes=64 * 1024 * 1024),
    )(xl, w1.T, w2)
    return out.reshape(H, C // TILE, w_tiles, TILE, LANES).transpose(0, 2, 4, 1, 3).reshape(B, H, W, C)
```

```python
import functools

import jax
import jax.numpy as jnp
import numpy as np
from jax import lax
import jax.experimental.pallas as pl
import jax.experimental.pallas.tpu as pltpu

LANES = 128
TILE = 8
RUN = 64
SEG_BITS = 6
SEG = 1 << SEG_BITS
BULK_AHEAD = 8
SMALL_AHEAD = 5
SMALL_PIECES = 4
EARLY_SLABS = 4
WR_SEGS = 6
FIRST_RUNS = 2


def _rows(g, k=0, n=RUN):
    start = g * RUN + k * n
    return pl.ds(start if isinstance(start, int) else pl.multiple_of(start, n), n)


def _wrap(i, n):
    return jnp.where(i >= n, i - n, i)


def _round(v):
    return v.astype(jnp.bfloat16).astype(jnp.float32)


def _cbam_kernel(x_hbm, w1t_hbm, w2_hbm, o_hbm,
                 buf, w1t_buf, w2_buf, w1_ref, w2t_ref, sum_ref, max_ref, gate_ref,
                 *, n_pixels, w_tiles):
    f32 = jnp.float32
    hidden, C = w2_hbm.shape
    nq = gate_ref.shape[0]

    def groups(q):
        return [(q * (RUN // TILE) + t) // w_tiles for t in range(RUN // TILE)]

    def pooler(runs_per_slab):
        partial = {}

        def fold(q, run):
            run, done = run.astype(f32), []
            for t, grp in enumerate(groups(q)):
                s, m, n = partial.pop(grp, None) or (sum_ref[grp], max_ref[grp], 0)
                tile = run[t * TILE:(t + 1) * TILE]
                s, m, n = s + tile, jnp.maximum(m, tile), n + 1
                if n == runs_per_slab * w_tiles:
                    done.append((grp, s, m))
                else:
                    partial[grp] = s, m, n
            return done

        return fold

    def read_and_pool(sems, w_sem):
        n_steps = buf.shape[0] // nq * SEG

        def locate(i):
            block = (i >> (SEG_BITS + 1)) * 2 + (i & 1)
            return block * nq, (i >> 1) & (SEG - 1)

        def fetch(segs, rows, slot):
            return pltpu.make_async_copy(x_hbm.at[segs, rows], buf.at[segs, rows], sems.at[slot])

        def start_bulk(i, slot):
            u, g = locate(i)
            fetch(pl.ds(u, nq - 1), _rows(g), slot).start(priority=1)

        def start_small(i, slot, k):
            u, g = locate(i)
            fetch(u + nq - 1, _rows(g, k, RUN // SMALL_PIECES), slot).start(priority=0)

        def first_small(j, _):
            i = lax.div(j, SMALL_PIECES)
            start_small(i, i, lax.rem(j, SMALL_PIECES))

        w_copies = [pltpu.make_async_copy(w1t_hbm, w1t_buf, w_sem),
                    pltpu.make_async_copy(w2_hbm, w2_buf, w_sem)]
        for copy in w_copies:
            copy.start()
        lax.fori_loop(0, BULK_AHEAD, lambda i, _: start_bulk(i, i), None)
        lax.fori_loop(0, SMALL_AHEAD * SMALL_PIECES, first_small, None)

        sum_ref[...] = jnp.zeros(sum_ref.shape, f32)
        max_ref[...] = jnp.full(max_ref.shape, -jnp.inf, f32)
        for copy in w_copies:
            copy.wait()
        for src, dst in ((w1t_buf, w1_ref), (w2_buf, w2t_ref)):
            dst[...] = jnp.concatenate(
                [src[...].astype(f32), jnp.zeros((LANES - hidden, C), f32)]).T

        def step(i, carry, *, bulk, small):
            slot, seg0 = carry
            u, g = locate(i)
            fetch(pl.ds(u, nq), _rows(g), slot).wait()
            fold = pooler(1)
            for q in range(nq):
                for k in range(SMALL_PIECES):
                    if small and q == k * (nq - 1) // (SMALL_PIECES - 1):
                        start_small(i + SMALL_AHEAD, _wrap(slot + SMALL_AHEAD, BULK_AHEAD), k)
                if bulk and q == nq - 1:
                    start_bulk(i + BULK_AHEAD, slot)
                for grp, s, m in fold(q, buf[u + _wrap(seg0 + q, nq), _rows(g)]):
                    sum_ref[grp], max_ref[grp] = s, m
            next_seg0 = jnp.where(g == SEG - 1, 0, _wrap(seg0 + nq - 1, nq))
            return _wrap(slot + 1, BULK_AHEAD), jnp.where((i & 1) == 1, next_seg0, seg0)

        def steps(lo, hi, carry, **starts):
            return lax.fori_loop(lo, hi, functools.partial(step, **starts), carry)

        end = n_steps - 2
        last = [locate(i)[0] for i in (end, end + 1)]
        early = [(u, 0, EARLY_SLABS, BULK_AHEAD) for u in last]
        late = [(u, EARLY_SLABS, nq - 1, BULK_AHEAD + 1) for u in last]
        in_pieces = [(u, nq - 1, nq, (end + j) % BULK_AHEAD) for j, u in enumerate(last)]

        carry = steps(0, end - BULK_AHEAD, (np.int32(0), np.int32(0)), bulk=True, small=True)
        for u, q0, q1, slot in early + late:
            fetch(pl.ds(u + q0, q1 - q0), _rows(SEG - 1), slot).start(priority=1)
        carry = steps(end - BULK_AHEAD, n_steps - SMALL_AHEAD, carry, bulk=False, small=True)
        steps(n_steps - SMALL_AHEAD, end, carry, bulk=False, small=False)

        h_avg = h_max = jnp.zeros((TILE, LANES), f32)
        fold = pooler(len(last))
        for stage in (in_pieces + early, late):
            for u, q0, q1, slot in stage:
                fetch(pl.ds(u + q0, q1 - q0), _rows(SEG - 1), slot).wait()
            for q, u in sorted((q, u) for u, q0, q1, _ in stage for q in range(q0, q1)):
                for grp, s, m in fold(q, buf[u + q, _rows(SEG - 1)]):
                    w1 = w1_ref[grp * TILE:(grp + 1) * TILE]
                    h_avg += _round(jnp.sum(s, axis=1, keepdims=True) * (1.0 / n_pixels)) * w1
                    h_max += jnp.max(m, axis=1, keepdims=True) * w1

        def relu(h):
            h = _round(jnp.sum(h, axis=0, keepdims=True))
            return h * (h > 0).astype(f32)

        lane = lax.broadcasted_iota(jnp.int32, (1, LANES), 1)
        h = jnp.where(lane < hidden, relu(h_avg) + relu(h_max), 0.0)
        return [jnp.sum(w2t_ref[grp * TILE:(grp + 1) * TILE] * h, axis=1, keepdims=True)
                for grp in range(C // TILE)]

    def to_gates(logits):
        return [jnp.broadcast_to(_round(jax.nn.sigmoid(z)), (TILE, LANES)) for z in logits]

    def slab_gate(gates, q):
        return jnp.concatenate([gates[grp] for grp in groups(q)])

    def scale(u, g, gate):
        buf[u, _rows(g)] = (buf[u, _rows(g)].astype(f32) * gate).astype(buf.dtype)

    def run_all(o_sem):
        def store(segs, g):
            pltpu.make_async_copy(
                buf.at[segs, _rows(g)], o_hbm.at[segs, _rows(g)], o_sem).start(priority=1)

        def send_run0(segs, gates):
            for u in segs:
                scale(u, 0, slab_gate(gates, u % nq))
                store(u, 0)

        def read_and_start_writing(*sems):
            logits = read_and_pool(*sems)
            gates = to_gates(logits[:groups(FIRST_RUNS - 1)[-1] + 1])
            send_run0(range(FIRST_RUNS), gates)
            return gates, logits[len(gates):]

        gates, logits = pl.run_scoped(
            read_and_start_writing,
            pltpu.SemaphoreType.DMA((BULK_AHEAD + 2,)), pltpu.SemaphoreType.DMA(()))
        gates = gates + to_gates(logits)
        send_run0(range(FIRST_RUNS, WR_SEGS), gates)
        for q in range(nq):
            gate_ref[q] = slab_gate(gates, q)

        def write_step(i, q):
            u, g = (i >> SEG_BITS) * WR_SEGS, i & (SEG - 1)
            for j in range(WR_SEGS):
                scale(u + j, g, gate_ref[_wrap(q + j, nq)])
            store(pl.ds(u, WR_SEGS), g)
            return _wrap(q + jnp.where(g == SEG - 1, WR_SEGS, 1), nq)

        lax.fori_loop(1, buf.shape[0] // WR_SEGS * SEG, write_step, np.int32(1))
        pltpu.make_async_copy(buf, o_hbm, o_sem).wait()

    pl.run_scoped(run_all, pltpu.SemaphoreType.DMA(()))


@jax.jit
def pallas_standalone__channel_attn_cbam__vision_kernel(
    x: jax.Array,
    w1: jax.Array,
    w2: jax.Array,
):
    B, H, W, C = x.shape
    hidden = w1.shape[1]
    w_tiles = W // LANES
    nq = C * w_tiles // RUN
    n_segs = H * nq // SEG
    assert B == 1 and W % LANES == 0 and C % TILE == 0 and C * w_tiles % RUN == 0
    assert SEG % nq == 1 and H % (2 * SEG) == 0 and n_segs % WR_SEGS == 0
    assert hidden <= LANES and WR_SEGS <= nq
    view = (n_segs, SEG * RUN, LANES)

    tiles = x.reshape(H, w_tiles, LANES, C // TILE, TILE).transpose(0, 3, 1, 4, 2)
    hbm = pl.BlockSpec(memory_space=pltpu.HBM)
    out = pl.pallas_call(
        functools.partial(_cbam_kernel, n_pixels=H * W, w_tiles=w_tiles),
        out_shape=jax.ShapeDtypeStruct(view, x.dtype),
        in_specs=[hbm, hbm, hbm],
        out_specs=hbm,
        scratch_shapes=[
            pltpu.VMEM(view, x.dtype),
            pltpu.VMEM((hidden, C), w1.dtype),
            pltpu.VMEM((hidden, C), w2.dtype),
            pltpu.VMEM((C, LANES), jnp.float32),
            pltpu.VMEM((C, LANES), jnp.float32),
            pltpu.VMEM((C // TILE, TILE, LANES), jnp.float32),
            pltpu.VMEM((C // TILE, TILE, LANES), jnp.float32),
            pltpu.VMEM((nq, RUN, LANES), jnp.float32),
        ],
        compiler_params=pltpu.CompilerParams(vmem_limit_bytes=64 * 1024 * 1024),
    )(tiles.reshape(view), w1.T, w2)
    return out.reshape(tiles.shape).transpose(0, 2, 4, 1, 3).reshape(B, H, W, C)
```

```python
import functools

import jax
import jax.numpy as jnp
import numpy as np
from jax import lax
import jax.experimental.pallas as pl
import jax.experimental.pallas.tpu as pltpu

LANES = 128
TILE = 8
RUN = 64
TILES_PER_RUN = RUN // TILE
SEG_BITS = 6
SEG = 1 << SEG_BITS
BULK_AHEAD = 8
SMALL_AHEAD = 5
SMALL_PIECES = 4
EARLY_SLABS = 4
WR_SEGS = 6
FIRST_RUNS = 2


def _rows(g, k=0, n=RUN):
    start = g * RUN + k * n
    return pl.ds(start if isinstance(start, int) else pl.multiple_of(start, n), n)


def _wrap(i, n):
    return jnp.where(i >= n, i - n, i)


def _round(v):
    return v.astype(jnp.bfloat16).astype(jnp.float32)


def _cbam_kernel(x_hbm, w1t_hbm, w2_hbm, o_hbm,
                 buf, w1t_buf, w2_buf, w1_ref, w2t_ref, sum_ref, max_ref, gate_ref,
                 *, n_pixels, w_tiles):
    f32 = jnp.float32
    hidden, C = w2_hbm.shape
    n_groups = C // TILE
    nq = n_groups * w_tiles // TILES_PER_RUN

    def pool(total, peak, runs, skip=0):
        tiles = runs.astype(f32).reshape(-1, TILE, LANES)[skip:skip + total.shape[0] * w_tiles]
        tiles = tiles.reshape(-1, w_tiles, TILE, LANES)
        for t in range(w_tiles):
            total, peak = total + tiles[:, t], jnp.maximum(peak, tiles[:, t])
        return total, peak

    def read_and_pool(sems, w_sem):
        n_steps = buf.shape[0] // nq * SEG

        def locate(i):
            block = (i >> (SEG_BITS + 1)) * 2 + (i & 1)
            return block * nq, (i >> 1) & (SEG - 1)

        def fetch(segs, rows, slot):
            return pltpu.make_async_copy(x_hbm.at[segs, rows], buf.at[segs, rows], sems.at[slot])

        def start_bulk(i, slot):
            u, g = locate(i)
            fetch(pl.ds(u, nq - 1), _rows(g), slot).start(priority=1)

        def start_small(i, slot, k):
            u, g = locate(i)
            fetch(u + nq - 1, _rows(g, k, RUN // SMALL_PIECES), slot).start(priority=0)

        def first_small(j, _):
            i = lax.div(j, SMALL_PIECES)
            start_small(i, i, lax.rem(j, SMALL_PIECES))

        w_copies = [pltpu.make_async_copy(w1t_hbm, w1t_buf, w_sem),
                    pltpu.make_async_copy(w2_hbm, w2_buf, w_sem)]
        for copy in w_copies:
            copy.start()
        lax.fori_loop(0, BULK_AHEAD, lambda i, _: start_bulk(i, i), None)
        lax.fori_loop(0, SMALL_AHEAD * SMALL_PIECES, first_small, None)

        sum_ref[...] = jnp.zeros(sum_ref.shape, f32)
        max_ref[...] = jnp.full(max_ref.shape, -jnp.inf, f32)
        for copy in w_copies:
            copy.wait()
        for src, dst in ((w1t_buf, w1_ref), (w2_buf, w2t_ref)):
            w = jnp.concatenate([src[...].astype(f32), jnp.zeros((LANES - hidden, C), f32)])
            dst[...] = w.T.reshape(dst.shape)

        def step(i, carry, *, bulk, small):
            slot, seg0 = carry
            u, g = locate(i)
            fetch(pl.ds(u, nq), _rows(g), slot).wait()
            runs = []
            for q in range(nq):
                for k in range(SMALL_PIECES):
                    if small and q == k * (nq - 1) // (SMALL_PIECES - 1):
                        start_small(i + SMALL_AHEAD, _wrap(slot + SMALL_AHEAD, BULK_AHEAD), k)
                runs.append(buf[u + _wrap(seg0 + q, nq), _rows(g)].astype(f32))
            if bulk:
                start_bulk(i + BULK_AHEAD, slot)
            sum_ref[...], max_ref[...] = pool(sum_ref[...], max_ref[...], jnp.concatenate(runs))
            next_seg0 = jnp.where(g == SEG - 1, 0, _wrap(seg0 + nq - 1, nq))
            return _wrap(slot + 1, BULK_AHEAD), jnp.where((i & 1) == 1, next_seg0, seg0)

        def steps(lo, hi, carry, **starts):
            return lax.fori_loop(lo, hi, functools.partial(step, **starts), carry)

        end = n_steps - 2
        last = [locate(i)[0] for i in (end, end + 1)]

        def fetch_last(q0, q1, slots):
            return [fetch(pl.ds(u + q0, q1 - q0), _rows(SEG - 1), slot)
                    for u, slot in zip(last, slots)]

        def layer1(g0, g1):
            q0, skip = divmod(g0 * w_tiles, TILES_PER_RUN)
            q1 = pl.cdiv(g1 * w_tiles, TILES_PER_RUN)
            total, peak = sum_ref[g0:g1], max_ref[g0:g1]
            for u in last:
                total, peak = pool(total, peak, buf[u + q0:u + q1, _rows(SEG - 1)], skip)
            avg = _round(jnp.sum(total, axis=2, keepdims=True) * (1.0 / n_pixels))
            top = jnp.max(peak, axis=2, keepdims=True)
            return [jnp.sum(v * w1_ref[g0:g1], axis=0) for v in (avg, top)]

        early = fetch_last(0, EARLY_SLABS, [BULK_AHEAD] * 2)
        late = fetch_last(EARLY_SLABS, nq - 1, [BULK_AHEAD + 1] * 2)
        in_pieces = fetch_last(nq - 1, nq, [end % BULK_AHEAD, (end + 1) % BULK_AHEAD])
        late_lo = EARLY_SLABS * TILES_PER_RUN // w_tiles
        late_hi = pl.cdiv((nq - 1) * TILES_PER_RUN, w_tiles)

        carry = steps(0, end - BULK_AHEAD, (np.int32(0), np.int32(0)), bulk=True, small=True)
        for copy in early + late:
            copy.start(priority=1)
        carry = steps(end - BULK_AHEAD, n_steps - SMALL_AHEAD, carry, bulk=False, small=True)
        steps(n_steps - SMALL_AHEAD, end, carry, bulk=False, small=False)
        for copy in in_pieces + early:
            copy.wait()
        h_early = [a + b for a, b in zip(layer1(0, late_lo), layer1(late_hi, n_groups))]
        for copy in late:
            copy.wait()
        h_avg, h_max = [_round(jnp.sum(a + b, axis=0, keepdims=True))
                        for a, b in zip(h_early, layer1(late_lo, late_hi))]

        h = h_avg * (h_avg > 0).astype(f32) + h_max * (h_max > 0).astype(f32)
        h = jnp.where(lax.broadcasted_iota(jnp.int32, h.shape, 1) < hidden, h, 0.0)
        return jnp.sum(w2t_ref[...] * h, axis=2, keepdims=True)

    def tile_gates(logits):
        gates = jax.nn.sigmoid(logits)[:, None]
        gates = jnp.broadcast_to(gates, (logits.shape[0], w_tiles, TILE, LANES))
        return gates.reshape(-1, LANES)

    def run_all(o_sem):
        def scale_and_store(segs, g, gates):
            buf[segs, _rows(g)] = buf[segs, _rows(g)] * gates.astype(buf.dtype)
            pltpu.make_async_copy(
                buf.at[segs, _rows(g)], o_hbm.at[segs, _rows(g)], o_sem).start(priority=1)

        n_first = pl.cdiv(FIRST_RUNS * TILES_PER_RUN, w_tiles)

        def read_and_start_writing(*sems):
            logits = read_and_pool(*sems)
            gates = tile_gates(logits[:n_first])
            for u in range(FIRST_RUNS):
                scale_and_store(u, 0, gates[u * RUN:(u + 1) * RUN])
            return gates, logits[n_first:]

        gates, logits = pl.run_scoped(
            read_and_start_writing,
            pltpu.SemaphoreType.DMA((BULK_AHEAD + 2,)), pltpu.SemaphoreType.DMA(()))
        gates = jnp.concatenate([gates, tile_gates(logits)]).reshape(nq, RUN, LANES)
        for u in range(FIRST_RUNS, WR_SEGS):
            scale_and_store(u, 0, gates[u])
        gate_ref[...] = jnp.concatenate([gates, gates[:WR_SEGS - 1]]).astype(gate_ref.dtype)

        def write_step(i, q):
            u, g = (i >> SEG_BITS) * WR_SEGS, i & (SEG - 1)
            scale_and_store(pl.ds(u, WR_SEGS), g, gate_ref[pl.ds(q, WR_SEGS)])
            return _wrap(q + jnp.where(g == SEG - 1, WR_SEGS, 1), nq)

        lax.fori_loop(1, buf.shape[0] // WR_SEGS * SEG, write_step, np.int32(1))
        pltpu.make_async_copy(buf, o_hbm, o_sem).wait()

    pl.run_scoped(run_all, pltpu.SemaphoreType.DMA(()))


@jax.jit
def pallas_standalone__channel_attn_cbam__vision_kernel(
    x: jax.Array,
    w1: jax.Array,
    w2: jax.Array,
):
    B, H, W, C = x.shape
    hidden = w1.shape[1]
    w_tiles = W // LANES
    nq = C * w_tiles // RUN
    n_segs = H * nq // SEG
    assert B == 1 and W % LANES == 0 and C % TILE == 0 and C * w_tiles % RUN == 0
    assert SEG % nq == 1 and H % (2 * SEG) == 0 and n_segs % WR_SEGS == 0
    assert hidden <= LANES and WR_SEGS <= nq
    view = (n_segs, SEG * RUN, LANES)
    per_channel = pltpu.VMEM((C // TILE, TILE, LANES), jnp.float32)

    tiles = x.reshape(H, w_tiles, LANES, C // TILE, TILE).transpose(0, 3, 1, 4, 2)
    hbm = pl.BlockSpec(memory_space=pltpu.HBM)
    out = pl.pallas_call(
        functools.partial(_cbam_kernel, n_pixels=H * W, w_tiles=w_tiles),
        out_shape=jax.ShapeDtypeStruct(view, x.dtype),
        in_specs=[hbm, hbm, hbm],
        out_specs=hbm,
        scratch_shapes=[
            pltpu.VMEM(view, x.dtype),
            pltpu.VMEM((hidden, C), w1.dtype),
            pltpu.VMEM((hidden, C), w2.dtype),
            per_channel, per_channel, per_channel, per_channel,
            pltpu.VMEM((nq + WR_SEGS - 1, RUN, LANES), x.dtype),
        ],
        compiler_params=pltpu.CompilerParams(vmem_limit_bytes=64 * 1024 * 1024),
        name="cbam_channel_attention",
    )(tiles.reshape(view), w1.T, w2)
    return out.reshape(tiles.shape).transpose(0, 2, 4, 1, 3).reshape(B, H, W, C)
```
